```python
import os as _os
_os.environ.setdefault("JAX_PLATFORMS", "cpu")
import jax
import jax.numpy as jnp

def _softmax(x, axis=-1):
    return jax.nn.softmax(x, axis=axis)
def _gelu(x):
    return jax.nn.gelu(x, approximate=True)
def _silu(x):
    return jax.nn.silu(x)
def _sigmoid(x):
    return jax.nn.sigmoid(x)
def _layernorm(x, axis=-1, eps=1e-5):
    m = jnp.mean(x, axis=axis, keepdims=True)
    v = jnp.var(x, axis=axis, keepdims=True)
    return (x - m) / jnp.sqrt(v + eps)
def _scatter_add(tgt, idx, src, axis=0):
    return tgt.at[idx].add(src)
def _segment_sum(src, seg, n):
    return jax.ops.segment_sum(src, seg, n)
class _Rng:
    def __init__(self, key):
        self._k = key
    def _next(self):
        self._k, sub = jax.random.split(self._k)
        return sub
    def normal(self, shape):
        return jax.random.normal(self._next(), shape, dtype=jnp.bfloat16)
    def randint(self, lo, hi, shape):
        return jax.random.randint(self._next(), shape, lo, hi, dtype=jnp.int32)
    def uniform(self, shape, lo=0.0, hi=1.0):
        return jax.random.uniform(self._next(), shape, jnp.bfloat16, lo, hi)
    def permutation(self, n):
        return jax.random.permutation(self._next(), n)


kernel_name = 'gated_mix__linear_attn_block__mixer_s_mlp__prompt'

def setup_inputs():
    _rng = _Rng(jax.random.key(int.from_bytes(__import__("os").urandom(4), "little")))
    _w = (lambda a: (lambda t: t.astype(jnp.bfloat16) if jnp.issubdtype(t.dtype, jnp.floating) else t)(jnp.asarray(a)))
    def _A_setup():
        B, S, D = 1, 2048, 640
        return {
            "x": _w((lambda *s: _rng.normal(s) * 0.05)(B, S, D)),
            "wqkv": _w((lambda *s: _rng.normal(s) * 0.8)(D, 3 * D)),
            "wo": _w((lambda *s: _rng.normal(s) * 0.1)(D, D)),
        }
    _A_in = _A_setup()

    def _B_setup():
        B, S, D, F = 1, 2048, 640, 1728
        return {
            "x":  _w((lambda *s: _rng.normal(s) * 0.05)(B, S, D)),
            "w1": _w((lambda *s: _rng.normal(s) * 0.2)(D, D) * (D ** -0.5)),
            "w2": _w((lambda *s: _rng.normal(s) * 0.2)(D, D) * (D ** -0.5)),
            "w3": _w((lambda *s: _rng.normal(s) * 0.2)(D, F) * (D ** -0.5)),
            "w4": _w((lambda *s: _rng.normal(s) * 0.2)(F, D) * (F ** -0.5)),
        }
    _B_in = _B_setup()

    return {
        "A_x": _A_in["x"],
        "A_wqkv": _A_in["wqkv"],
        "A_wo": _A_in["wo"],
        "B_x": _B_in["x"],
        "B_w1": _B_in["w1"],
        "B_w2": _B_in["w2"],
        "B_w3": _B_in["w3"],
        "B_w4": _B_in["w4"],
        "gate_w": _w((lambda *s: _rng.normal(s) * 0.05)(640) * 16.0),
    }

def reference(A_x, A_wqkv, A_wo, B_x, B_w1, B_w2, B_w3, B_w4, gate_w):
    def _A_ref(x, wqkv, wo):
        B, S, D = x.shape
        H = 32; Dh = D // H
        qkv = (lambda x, *d: x.transpose(*d))((x @ wqkv).reshape(B, S, 3, H, Dh), 2, 0, 3, 1, 4)
        q, k, v = qkv[0], qkv[1], qkv[2]
        phi = lambda t: jnp.where(t > 0, t + 1, jnp.exp(t)) + 1e-6
        pq, pk = phi(q), phi(k)
        kv = jnp.einsum("bhsd,bhse->bhde", pk, v)
        z = jnp.einsum("bhsd->bhd", pk)
        num = jnp.einsum("bhqd,bhde->bhqe", pq, kv)
        den = jnp.einsum("bhqd,bhd->bhq", pq, z)[..., None] + 1e-6
        o = num / den
        return (lambda x, *d: x.transpose(*d))(o, 0, 2, 1, 3).reshape(B, S, D) @ wo

    def _B_ref(x, w1, w2, w3, w4):
        B, S, D = x.shape
        h = _gelu(_layernorm(x, axis=-1) @ w1)
        c = D // 4
        g0 = jnp.pad(h[:, :, 0*c:1*c], ((0, 0), (1, 0), (0, 0)))[:, :S, :]
        g1 = jnp.pad(h[:, :, 1*c:2*c], ((0, 0), (0, 1), (0, 0)))[:, 1:, :]
        g2 = jnp.pad(h[:, :, 2*c:3*c], ((0, 0), (2, 0), (0, 0)))[:, :S, :]
        g3 = jnp.pad(h[:, :, 3*c:   ], ((0, 0), (0, 2), (0, 0)))[:, 2:, :]
        hs = jnp.concatenate([g0, g1, g2, g3], axis=-1) @ w2
        x1 = x + hs
        h2 = _gelu(_layernorm(x1, axis=-1) @ w3) @ w4
        return x1 + h2

    x = A_x
    g = _sigmoid((x * gate_w).sum(-1, keepdims=True))
    a = _A_ref(x, A_wqkv, A_wo)
    b = _B_ref(x, B_w1, B_w2, B_w3, B_w4)
    return g * a + (1 - g) * b
```

```python
import functools
import jax
import jax.numpy as jnp
import jax.experimental.pallas as pl
import jax.experimental.pallas.tpu as pltpu

S, D, F, H, DH = 2048, 640, 1728, 32, 20
LANE = 128
NJ = D // LANE
BF = jnp.bfloat16
F32 = jnp.float32

def _bands():
    out = []
    off = 0
    for j in range(NJ):
        h_lo = (LANE * j) // DH
        h_hi = (LANE * (j + 1) - 1) // DH
        lo = (h_lo * DH) // 16 * 16
        hi = -(-((h_hi + 1) * DH) // 16) * 16
        out.append((lo, hi, off))
        off += hi - lo
    return out, off
BANDS, BAND_ROWS = _bands()


def _head_of(idx):
    return (idx * 3277) >> 16


def _gelu(x):
    c = 0.7978845608028654
    return 0.5 * x * (1.0 + jnp.tanh(c * (x + 0.044715 * (x * x * x))))


def _phi(t):
    return jnp.where(t > 0, t + 1.0, jnp.exp(t)) + 1e-6


def _ln(x):
    m = jnp.mean(x, axis=-1, keepdims=True)
    xc = x - m
    v = jnp.mean(xc * xc, axis=-1, keepdims=True)
    return xc * jax.lax.rsqrt(v + 1e-5)


def _dot(a, b):
    return jnp.dot(a, b, preferred_element_type=F32)


def _dot_nt(a, b):
    return jax.lax.dot_general(a, b, (((1,), (1,)), ((), ())), preferred_element_type=F32)


def make(T1=256, T2=256):
    N1 = S // T1
    N2 = S // T2

    def kernel(xa_hbm, wqkv_hbm, wo_hbm, w1_hbm, w2_hbm, w3_hbm, w4_hbm, gw_ref,
               out_hbm,
               xa_v, wq_v, wk_v, wv_v, wo_v, w1_v, w2_v, w3_v, w4_v,
               h_v, wkt_v, kv_acc, z_acc, m32_v, m_v, zmat_v, e_v, obuf,
               wsem, xasem, osem):
        def xa_cp(t):
            return pltpu.make_async_copy(xa_hbm.at[pl.ds(t * T1, T1)], xa_v.at[pl.ds(t * T1, T1)], xasem.at[t])
        wcp = {}
        for i, (nm, src, dst) in enumerate([
                ("wq", wqkv_hbm.at[:, pl.ds(0, D)], wq_v), ("wk", wqkv_hbm.at[:, pl.ds(D, D)], wk_v),
                ("wv", wqkv_hbm.at[:, pl.ds(2 * D, D)], wv_v),
                ("w1", w1_hbm, w1_v), ("wo", wo_hbm, wo_v),
                ("w2", w2_hbm, w2_v), ("w3", w3_hbm, w3_v), ("w4", w4_hbm, w4_v)]):
            wcp[nm] = pltpu.make_async_copy(src, dst, wsem.at[i])
        wcp["wk"].start()
        xa_cp(0).start()
        wcp["wv"].start()
        wcp["w1"].start()

        h_v[pl.ds(0, 8), :] = jnp.zeros((8, D), F32)
        h_v[pl.ds(S + 8, 8), :] = jnp.zeros((8, D), F32)
        kv_acc[...] = jnp.zeros(kv_acc.shape, F32)
        z_acc[...] = jnp.zeros(z_acc.shape, F32)
        er = jax.lax.broadcasted_iota(jnp.int32, (LANE, D), 0)
        ec = jax.lax.broadcasted_iota(jnp.int32, (LANE, D), 1)
        e_v[...] = jnp.where((er < 64) & ((er & 31) == _head_of(ec)), 1.0, 0.0).astype(BF)

        wcp["wk"].wait()
        for t in range(1, N1):
            xa_cp(t).start()
        for nm in ["wq", "wo", "w2", "w3", "w4"]:
            wcp[nm].start()
        ir = jax.lax.broadcasted_iota(jnp.int32, (LANE, LANE), 0)
        ic = jax.lax.broadcasted_iota(jnp.int32, (LANE, LANE), 1)
        eye = jnp.where(ir == ic, 1.0, 0.0).astype(BF)
        for i in range(NJ):
            wkt_v[pl.ds(i * LANE, LANE), :] = _dot_nt(eye, wk_v[:, pl.ds(i * LANE, LANE)]).astype(BF)
        wcp["wv"].wait()
        wcp["w1"].wait()

        def phase1(t, carry):
            r0 = pl.multiple_of(t * T1, T1)
            xa_cp(t).wait()
            xa = xa_v[pl.ds(r0, T1), :]
            pkt = _phi(_dot_nt(wkt_v[...], xa))
            v = _dot(xa, wv_v[...]).astype(BF)
            h = _gelu(_dot(_ln(xa.astype(F32)).astype(BF), w1_v[...]))
            h_v[pl.ds(r0 + 8, T1), :] = h
            zs = pkt[:, 0:LANE]
            for c in range(1, T1 // LANE):
                zs = zs + pkt[:, c * LANE:(c + 1) * LANE]
            z_acc[...] += zs
            pkt = pkt.astype(BF)
            for j, (lo, hi, off) in enumerate(BANDS):
                kv_acc[pl.ds(off, hi - lo), :] += _dot(pkt[lo:hi, :], v[:, j * LANE:(j + 1) * LANE])
            return carry
        jax.lax.fori_loop(0, N1, phase1, 0)

        wcp["wo"].wait()
        wcp["wq"].wait()
        wcp["w2"].wait()
        wcp["w3"].wait()
        wcp["w4"].wait()
        m32_v[...] = jnp.zeros(m32_v.shape, F32)
        for j, (lo, hi, off) in enumerate(BANDS):
            n = hi - lo
            rr = jax.lax.broadcasted_iota(jnp.int32, (n, LANE), 0) + lo
            cc = jax.lax.broadcasted_iota(jnp.int32, (n, LANE), 1) + j * LANE
            kvm = jnp.where(_head_of(rr) == _head_of(cc), kv_acc[pl.ds(off, n), :], 0.0).astype(BF)
            m32_v[pl.ds(lo, n), :] += _dot(kvm, wo_v[pl.ds(j * LANE, LANE), :])
        m_v[...] = m32_v[...].astype(BF)
        z = jnp.sum(z_acc[...], axis=1, keepdims=True)
        zr = jax.lax.broadcasted_iota(jnp.int32, (D, LANE), 0)
        zc = jax.lax.broadcasted_iota(jnp.int32, (D, LANE), 1)
        zmat_v[...] = jnp.where((zc < 64) & ((zc & 31) == _head_of(zr)), z, 0.0).astype(BF)

        def out_cp(t, slot):
            return pltpu.make_async_copy(obuf.at[slot], out_hbm.at[pl.ds(t * T2, T2)], osem.at[slot])

        lane = jax.lax.broadcasted_iota(jnp.int32, (T2, LANE), 1)

        def phase2(t, carry):
            r0 = pl.multiple_of(t * T2, T2)
            slot = t % 2
            @pl.when(t >= 2)
            def _():
                out_cp(t - 2, slot).wait()
            xa = xa_v[pl.ds(r0, T2), :]
            q = _dot(xa, wq_v[...])
            w = h_v[pl.ds(r0, T2 + 16), :]
            def sh(k, j):
                return w[8 + k:8 + k + T2, j * LANE:(j + 1) * LANE]
            hs = jnp.concatenate([
                sh(-1, 0),
                jnp.where(lane < 32, sh(-1, 1), sh(1, 1)),
                jnp.where(lane < 64, sh(1, 2), sh(-2, 2)),
                jnp.where(lane < 96, sh(-2, 3), sh(2, 3)),
                sh(2, 4)], axis=1).astype(BF)
            x1 = xa.astype(F32) + _dot(hs, w2_v[...])
            pq = _phi(q)
            den = _dot(pq.astype(BF), zmat_v[...]) + 1e-6
            r = 1.0 / den
            r_hi = r.astype(BF)
            r_lo = (r - r_hi.astype(F32)).astype(BF)
            rcat = jnp.where(lane < 32, r_hi, r_lo)
            rexp = _dot(rcat, e_v[...])
            h3 = _gelu(_dot_nt(_ln(x1).astype(BF), w3_v[...])).astype(BF)
            a = _dot((pq * rexp).astype(BF), m_v[...])
            g = jax.nn.sigmoid(jnp.sum(xa.astype(F32) * gw_ref[...].astype(F32), axis=-1, keepdims=True))
            b = x1 + _dot(h3, w4_v[...])
            res = (b + g * (a - b)).astype(BF)
            obuf[slot] = res
            out_cp(t, slot).start()
            return carry
        jax.lax.fori_loop(0, N2, phase2, 0)
        out_cp(N2 - 2, (N2 - 2) % 2).wait()
        out_cp(N2 - 1, (N2 - 1) % 2).wait()

    @jax.jit
    def fn(A_x, A_wqkv, A_wo, B_x, B_w1, B_w2, B_w3, B_w4, gate_w):
        any_spec = pl.BlockSpec(memory_space=pltpu.HBM)
        out = pl.pallas_call(
            kernel,
            out_shape=jax.ShapeDtypeStruct((S, D), BF),
            in_specs=[any_spec] * 7 + [pl.BlockSpec(memory_space=pltpu.VMEM)],
            out_specs=any_spec,
            scratch_shapes=[
                pltpu.VMEM((S, D), BF),
                pltpu.VMEM((D, D), BF), pltpu.VMEM((D, D), BF), pltpu.VMEM((D, D), BF),
                pltpu.VMEM((D, D), BF), pltpu.VMEM((D, D), BF), pltpu.VMEM((D, D), BF),
                pltpu.VMEM((F, D), BF), pltpu.VMEM((F, D), BF),
                pltpu.VMEM((S + 16, D), F32), pltpu.VMEM((D, D), BF),
                pltpu.VMEM((BAND_ROWS, LANE), F32), pltpu.VMEM((D, LANE), F32),
                pltpu.VMEM((D, D), F32), pltpu.VMEM((D, D), BF), pltpu.VMEM((D, LANE), BF), pltpu.VMEM((LANE, D), BF),
                pltpu.VMEM((2, T2, D), BF),
                pltpu.SemaphoreType.DMA((8,)), pltpu.SemaphoreType.DMA((N1,)),
                pltpu.SemaphoreType.DMA((2,)),
            ],
            compiler_params=pltpu.CompilerParams(vmem_limit_bytes=100 * 1024 * 1024),
            name="gmix",
        )(A_x.reshape(S, D), A_wqkv, A_wo, B_w1, B_w2, B_w3.T, B_w4, gate_w.reshape(1, D))
        return out.reshape(1, S, D)
    return fn


pallas_gated_mix__linear_attn_block__mixer_s_mlp__prompt_kernel = make()
```

```python
import functools
import jax
import jax.numpy as jnp
import jax.experimental.pallas as pl
import jax.experimental.pallas.tpu as pltpu

S, D, F, H, DH = 2048, 640, 1728, 32, 20
LANE = 128
NJ = D // LANE
FM = (F // LANE) * LANE
BF = jnp.bfloat16
F32 = jnp.float32
HP = 32
LAG = 16


def _bands():
    out = []
    for j in range(NJ):
        h_lo = (LANE * j) // DH
        h_hi = (LANE * (j + 1) - 1) // DH
        lo = (h_lo * DH) // 16 * 16
        hi = -(-((h_hi + 1) * DH) // 16) * 16
        out.append((lo, hi))
    return out
BANDS = _bands()


def _head_of(idx):
    return (idx * 3277) >> 16


def _gelu(x):
    c = 0.7978845608028654
    hx = 0.5 * x
    u = x * (c + (c * 0.044715) * (x * x))
    return hx + hx * jnp.tanh(u)


def _phi(t):
    return jnp.where(t > 0, t + 1.0, jnp.exp(t)) + 1e-6


def _sigmoid(x):
    return 0.5 + 0.5 * jnp.tanh(0.5 * x)


def _dot(a, b):
    return jnp.dot(a, b, preferred_element_type=F32)


def _dot_nt(a, b):
    return jax.lax.dot_general(a, b, (((1,), (1,)), ((), ())), preferred_element_type=F32)


def _dot_tn(a, b):
    return jax.lax.dot_general(a, b, (((0,), (0,)), ((), ())), preferred_element_type=F32)


def _lane_tiles_sum(x):
    acc = x[:, 0:LANE]
    for j in range(1, x.shape[1] // LANE):
        acc = acc + x[:, j * LANE:(j + 1) * LANE]
    return acc


def make(T1=256, T2=1024, order2="q,phi,w2,ln,a,w3,w4", order1="k,h,g,hs", first_order="h,k,g,hs", ocols=True, mean1=False, hs1=False, gate1=True, biglag=False, orows=256):
    N1 = S // T1
    N2 = S // T2
    order2 = order2.split(",")
    order1 = order1.split(",")
    first_order = first_order.split(",")

    def kernel(xa_hbm, wqkv_hbm, wo_hbm, w1_hbm, w2_hbm, w3_hbm, w4_hbm, gw_hbm,
               out_hbm,
               xa_v, wq_v, wk_v, wv_v, wo_v, w1_v, w2_v, w3_v, w4_v,
               gw_ref, w2rs_v, h_v, hsb_v, g_v, mx_v, wqt_v, g_acc, z_acc, m_v, zb_v, obuf,
               wsem, osem):
        def xa_cp(t):
            return pltpu.make_async_copy(xa_hbm.at[pl.ds(t * T1, T1)], xa_v.at[pl.ds(t * T1, T1)], wsem.at[9 + t])
        wcp = {}
        for i, (nm, src, dst) in enumerate([
                ("wq", wqkv_hbm.at[:, pl.ds(0, D)], wq_v), ("wk", wqkv_hbm.at[:, pl.ds(D, D)], wk_v),
                ("wv", wqkv_hbm.at[:, pl.ds(2 * D, D)], wv_v),
                ("w1", w1_hbm, w1_v), ("wo", wo_hbm, wo_v),
                ("w2", w2_hbm, w2_v), ("w3", w3_hbm, w3_v), ("w4", w4_hbm, w4_v), ("gw", gw_hbm, gw_ref)]):
            wcp[nm] = pltpu.make_async_copy(src, dst, wsem.at[i])
        wcp["gw"].start()
        xa_cp(0).start()
        wcp["w1"].start()
        wcp["wk"].start()
        if mean1:
            wcp["w2"].start()
        for t in range(1, N1):
            xa_cp(t).start()
        for nm in ["wv", "wo", "wq", "w2", "w3", "w4"]:
            if not (mean1 and nm == "w2"):
                wcp[nm].start()

        h_v[pl.ds(0, HP), :] = jnp.zeros((HP, D), F32)
        h_v[pl.ds(HP + S, 8), :] = jnp.zeros((8, D), F32)

        def shifted(r, n):
            w = h_v[pl.ds(HP + r - 8, n + 16), :]
            lane = jax.lax.broadcasted_iota(jnp.int32, (n, LANE), 1)
            cache = {}
            def sh(k, j):
                if (k, j) not in cache:
                    cache[(k, j)] = pltpu.roll(w[:, j * LANE:(j + 1) * LANE], (-k) % (n + 16), 0)[8:8 + n]
                return cache[(k, j)]
            return jnp.concatenate([
                sh(-1, 0),
                jnp.where(lane < 32, sh(-1, 1), sh(1, 1)),
                jnp.where(lane < 64, sh(1, 2), sh(-2, 2)),
                jnp.where(lane < 96, sh(-2, 3), sh(2, 3)),
                sh(2, 4)], axis=1)

        def hs_store(r, n):
            hs = shifted(r, n)
            hsb_v[pl.ds(r + LAG, n), :] = hs.astype(BF)
            if mean1:
                u = jnp.sum(_lane_tiles_sum(hs * w2rs_v[0:1, :]), axis=-1, keepdims=True) * (1.0 / D)
                mx_v[pl.ds(r + LAG, n), :] = mx_v[pl.ds(r + LAG, n), :] + u

        def gate(xf):
            gw = gw_ref[...].astype(F32)
            acc = xf[:, 0:LANE] * gw[0:1, :]
            for j in range(1, NJ):
                acc = acc + xf[:, j * LANE:(j + 1) * LANE] * gw[j:j + 1, :]
            return _sigmoid(jnp.sum(acc, axis=-1, keepdims=True))

        def phase1(t, first):
            r0 = t * T1 if isinstance(t, int) else pl.multiple_of(t * T1, T1)
            xa_cp(t).wait()
            if first:
                wcp["gw"].wait()
            xa = xa_v[pl.ds(r0, T1), :]
            st = {}
            def mm(a, b):
                if first:
                    hh = T1 // 2
                    return jnp.concatenate([_dot(a[:hh], b), _dot(a[hh:], b)], axis=0)
                return _dot(a, b)
            def f_k():
                if first:
                    wcp["wk"].wait()
                pk = _phi(mm(xa, wk_v[...]))
                zs = jnp.sum(pk.reshape(T1 // 8, 8, D), axis=0)
                if first:
                    z_acc[...] = zs
                else:
                    z_acc[...] += zs
                st["pkt"] = pk.astype(BF).T
            def f_h():
                xf = xa.astype(F32)
                m = jnp.sum(_lane_tiles_sum(xf), axis=-1, keepdims=True) * (1.0 / D)
                xc = xf - m
                v = jnp.sum(_lane_tiles_sum(xc * xc), axis=-1, keepdims=True) * (1.0 / D)
                rs = jax.lax.rsqrt(v + 1e-5)
                ln = (xf * rs - m * rs).astype(BF)
                if gate1:
                    g_v[pl.ds(r0, T1), :] = jnp.broadcast_to(gate(xf), (T1, LANE))
                mx_v[pl.ds(r0 + LAG, T1), :] = jnp.broadcast_to(m, (T1, LANE))
                if first:
                    wcp["w1"].wait()
                h_v[pl.ds(HP + r0, T1), :] = _gelu(mm(ln, w1_v[...]))
            def f_g():
                if first and mean1:
                    wcp["w2"].wait()
                gg = _dot(st["pkt"], xa)
                if first:
                    g_acc[...] = gg
                else:
                    g_acc[...] += gg
                if first and mean1:
                    w2rs_v[...] = _dot_nt(jnp.ones((16, D), BF), w2_v[...])
                    mx_v[pl.ds(0, LAG), :] = jnp.zeros((LAG, LANE), F32)
            def f_hs():
                if not hs1:
                    return
                if biglag:
                    if first:
                        return
                    hs_store(pl.multiple_of(r0 - T1 - LAG, LAG), T1)
                    return
                rr = r0 - LAG if isinstance(r0, int) else pl.multiple_of(r0 - LAG, LAG)
                hs_store(rr, T1)
            fs = dict(k=f_k, h=f_h, g=f_g, hs=f_hs)
            for nm in (first_order if first else order1):
                fs[nm]()

        phase1(0, True)
        def body1(t, c):
            phase1(t, False)
            return c
        jax.lax.fori_loop(1, N1, body1, 0)

        for nm in ["wv", "wo", "wq", "w2", "w3", "w4"]:
            if not (mean1 and nm == "w2"):
                wcp[nm].wait()
        if hs1:
            if biglag:
                hs_store(S - T1 - LAG, T1 + LAG)
            else:
                hs_store(S - LAG, LAG)
        wqt_v[...] = wq_v[...].T
        kvms = []
        for j, (lo, hi) in enumerate(BANDS):
            n = hi - lo
            rr = jax.lax.broadcasted_iota(jnp.int32, (n, LANE), 0) + lo
            cc = jax.lax.broadcasted_iota(jnp.int32, (n, LANE), 1) + j * LANE
            kv = _dot(g_acc[pl.ds(lo, n), :].astype(BF), wv_v[:, pl.ds(j * LANE, LANE)])
            kvms.append(jnp.where(_head_of(rr) == _head_of(cc), kv, 0.0).astype(BF))
        parts = [_dot(kvms[j], wo_v[pl.ds(j * LANE, LANE), :]) for j in range(NJ)]
        edges = sorted(set([lo for lo, hi in BANDS] + [hi for lo, hi in BANDS]))
        for a, b in zip(edges[:-1], edges[1:]):
            acc = None
            for j, (lo, hi) in enumerate(BANDS):
                if lo <= a and b <= hi:
                    p = parts[j][a - lo:b - lo]
                    acc = p if acc is None else acc + p
            m_v[pl.ds(a, b - a), :] = acc.astype(BF)
        if not mean1:
            w2rs_v[...] = _dot_nt(jnp.ones((16, D), BF), w2_v[...])
        z = jnp.sum(z_acc[...], axis=0, keepdims=True)
        zb_v[...] = jnp.broadcast_to(z, (LANE, D)).T

        OR = min(orows, T2)
        OC = [(c * LANE, LANE, 0, T2) for c in range(NJ - 1)] + [((NJ - 1) * LANE, LANE, rr, OR) for rr in range(0, T2, OR)]
        def out_cp(t, c):
            c0, cn, rr, nr = OC[c]
            return pltpu.make_async_copy(obuf.at[pl.ds(t * T2 + rr, nr), pl.ds(c0, cn)], out_hbm.at[pl.ds(t * T2 + rr, nr), pl.ds(c0, cn)], osem.at[t * len(OC) + c])

        NP = H // 2
        sub = jax.lax.broadcasted_iota(jnp.int32, (NP, 8, T2), 1)

        def phase2(t, carry):
            r0 = pl.multiple_of(t * T2, T2)
            xa = xa_v[pl.ds(r0, T2), :]
            st = {}
            def f_q():
                st["q"] = _dot_nt(wqt_v[...], xa)
            def f_w2():
                hsb = hsb_v[pl.ds(r0 + LAG, T2), :] if hs1 else shifted(r0, T2).astype(BF)
                m = mx_v[pl.ds(r0 + LAG, T2), :]
                if not mean1:
                    u = jnp.sum(_lane_tiles_sum(hsb.astype(F32) * w2rs_v[0:1, :]), axis=-1, keepdims=True) * (1.0 / D)
                    m = m + u
                st["m"] = m
                m5 = jnp.concatenate([m] * NJ, axis=1)
                st["xc"] = (xa.astype(F32) - m5) + _dot(hsb, w2_v[...])
            def f_phi():
                pq = _phi(st["q"])
                zb = zb_v[...]
                tz = pq * jnp.concatenate([zb] * (T2 // LANE), axis=1)
                t4 = tz.reshape(NP, 5, 8, T2)
                p4 = pq.reshape(NP, 5, 8, T2)
                lo4 = sub < 4
                sa = t4[:, 0] + t4[:, 1] + jnp.where(lo4, t4[:, 2], 0.0)
                sb = t4[:, 3] + t4[:, 4] + jnp.where(lo4, 0.0, t4[:, 2])
                def allsum(a):
                    a = a + pltpu.roll(a, 4, 1)
                    a = a + pltpu.roll(a, 2, 1)
                    a = a + pltpu.roll(a, 1, 1)
                    return a
                da = allsum(sa) + 1e-6
                db = allsum(sb) + 1e-6
                def rc(d):
                    r = pl.reciprocal(d, approx=True)
                    return r * (2.0 - d * r)
                ra = rc(da); rb = rc(db)
                pn = jnp.stack([p4[:, 0] * ra, p4[:, 1] * ra, p4[:, 2] * jnp.where(lo4, ra, rb), p4[:, 3] * rb, p4[:, 4] * rb], axis=1)
                st["pqn"] = pn.reshape(D, T2).astype(BF)
            def f_ln():
                xc = st["xc"]
                st["ln"] = xc.astype(BF)
                st["rs"] = jax.lax.rsqrt(jnp.sum(_lane_tiles_sum(xc * xc), axis=-1, keepdims=True) * (1.0 / D) + 1e-5)
            def f_w3():
                h3l = _gelu(_dot_nt(w3_v[FM:F, :], st["ln"]).T * st["rs"]).astype(BF)
                h3m = _gelu(_dot_nt(st["ln"], w3_v[0:FM, :]) * st["rs"]).astype(BF)
                st["h3"] = jnp.concatenate([h3m, h3l], axis=1)
            def f_a():
                st["a"] = _dot_tn(st["pqn"], m_v[...])
            def f_w4():
                st["bm"] = st["xc"] + _dot(st["h3"], w4_v[...])
            fs = dict(q=f_q, w2=f_w2, phi=f_phi, ln=f_ln, w3=f_w3, a=f_a, w4=f_w4)
            for nm in order2:
                fs[nm]()
            g = g_v[pl.ds(r0, T2), :] if gate1 else jnp.broadcast_to(gate(xa.astype(F32)), (T2, LANE))
            for c, (c0, cn, rr, nr) in enumerate(OC):
                nrep = cn // LANE
                gq = g[rr:rr + nr]; mq = st["m"][rr:rr + nr]
                gg = gq if nrep == 1 else jnp.concatenate([gq] * nrep, axis=1)
                mm_ = mq if nrep == 1 else jnp.concatenate([mq] * nrep, axis=1)
                b = st["bm"][rr:rr + nr, c0:c0 + cn] + mm_
                obuf[pl.ds(r0 + rr, nr), pl.ds(c0, cn)] = (b + gg * (st["a"][rr:rr + nr, c0:c0 + cn] - b)).astype(BF)
                out_cp(t, c).start()
            return carry
        jax.lax.fori_loop(0, N2, phase2, 0)
        for t in range(N2):
            for c in range(len(OC)):
                out_cp(t, c).wait()

    @jax.jit
    def fn(A_x, A_wqkv, A_wo, B_x, B_w1, B_w2, B_w3, B_w4, gate_w):
        any_spec = pl.BlockSpec(memory_space=pltpu.HBM)
        out = pl.pallas_call(
            kernel,
            out_shape=jax.ShapeDtypeStruct((S, D), BF),
            in_specs=[any_spec] * 8,
            out_specs=any_spec,
            scratch_shapes=[
                pltpu.VMEM((S, D), BF),
                pltpu.VMEM((D, D), BF), pltpu.VMEM((D, D), BF), pltpu.VMEM((D, D), BF),
                pltpu.VMEM((D, D), BF), pltpu.VMEM((D, D), BF), pltpu.VMEM((D, D), BF),
                pltpu.VMEM((F, D), BF), pltpu.VMEM((F, D), BF),
                pltpu.VMEM((NJ, LANE), BF), pltpu.VMEM((16, D), F32),
                pltpu.VMEM((HP + S + 8, D), F32), pltpu.VMEM((S + LAG, D), BF),
                pltpu.VMEM((S, LANE), F32), pltpu.VMEM((S + LAG, LANE), F32),
                pltpu.VMEM((D, D), BF),
                pltpu.VMEM((D, D), F32), pltpu.VMEM((8, D), F32),
                pltpu.VMEM((D, D), BF), pltpu.VMEM((D, LANE), F32),
                pltpu.VMEM((S, D), BF),
                pltpu.SemaphoreType.DMA((9 + N1,)),
                pltpu.SemaphoreType.DMA((NJ * N2 + S // min(orows, T2),)),
            ],
            compiler_params=pltpu.CompilerParams(vmem_limit_bytes=100 * 1024 * 1024),
            name="gmix",
        )(A_x.reshape(S, D), A_wqkv, A_wo, B_w1, B_w2, B_w3.T, B_w4, gate_w.reshape(NJ, LANE))
        return out.reshape(1, S, D)
    return fn


pallas_gated_mix__linear_attn_block__mixer_s_mlp__prompt_kernel = make()
```

```python
import jax
import jax.numpy as jnp
import jax.experimental.pallas as pl
import jax.experimental.pallas.tpu as pltpu

S, D, F, H, DH = 2048, 640, 1728, 32, 20
LANE = 128
NJ = D // LANE
FM = (F // LANE) * LANE
BF = jnp.bfloat16
F32 = jnp.float32
HP = 8


def _bands():
    out = []
    for j in range(NJ):
        h_lo = (LANE * j) // DH
        h_hi = (LANE * (j + 1) - 1) // DH
        lo = (h_lo * DH) // 16 * 16
        hi = -(-((h_hi + 1) * DH) // 16) * 16
        out.append((lo, hi))
    return out
BANDS = _bands()


def _head_of(idx):
    return (idx * 3277) >> 16


def _gelu(x):
    c = 0.7978845608028654
    hx = 0.5 * x
    u = x * (c + (c * 0.044715) * (x * x))
    return hx + hx * jnp.tanh(u)


def _phi(t):
    return jnp.where(t > 0, t + 1.0, jnp.exp(t)) + 1e-6


def _sigmoid(x):
    return 0.5 + 0.5 * jnp.tanh(0.5 * x)


def _dot(a, b):
    return jnp.dot(a, b, preferred_element_type=F32)


def _dot_nt(a, b):
    return jax.lax.dot_general(a, b, (((1,), (1,)), ((), ())), preferred_element_type=F32)


def _dot_tn(a, b):
    return jax.lax.dot_general(a, b, (((0,), (0,)), ((), ())), preferred_element_type=F32)


def _lane_tiles_sum(x):
    acc = x[:, 0:LANE]
    for j in range(1, x.shape[1] // LANE):
        acc = acc + x[:, j * LANE:(j + 1) * LANE]
    return acc


def make(T0=256, T1=256, T2=1024, order2="q,phi,w2,ln,a,w3,w4", order1="k,h,g", first_order="h,k,g", orows=256, strided=True, gate1=True, defer_h0=False, ms=4, gs=2, gsl=1, zbv=1, wqloop=False, w2loop=True):
    N1 = (S - T0) // T1
    assert T0 + N1 * T1 == S
    N2 = S // T2
    order2 = order2.split(",")
    order1 = order1.split(",")
    first_order = first_order.split(",")
    NW = 9

    def kernel(xa_hbm, wqkv_hbm, wo_hbm, w1_hbm, w2_hbm, w3_hbm, w4_hbm, gw_hbm,
               out_hbm,
               xa_v, wq_v, wk_v, wv_v, wo_v, w1_v, w2_v, w3_v, w4_v,
               gw_ref, hpre_v, w2rs_v, h_v, g_v, mx_v, wqt_v, g_acc, z_acc, m_v, zb_v, obuf,
               wsem, osem):
        def xa_cp(t):
            if isinstance(t, int) and t < 0:
                return pltpu.make_async_copy(xa_hbm.at[pl.ds(0, T0)], xa_v.at[pl.ds(0, T0)], wsem.at[NW])
            return pltpu.make_async_copy(xa_hbm.at[pl.ds(T0 + t * T1, T1)], xa_v.at[pl.ds(T0 + t * T1, T1)], wsem.at[NW + 1 + t])
        wcp = {}
        for i, (nm, src, dst) in enumerate([
                ("wq", wqkv_hbm.at[:, pl.ds(0, D)], wq_v), ("wk", wqkv_hbm.at[:, pl.ds(D, D)], wk_v),
                ("wv", wqkv_hbm.at[:, pl.ds(2 * D, D)], wv_v),
                ("w1", w1_hbm, w1_v), ("wo", wo_hbm, wo_v),
                ("w2", w2_hbm, w2_v), ("w3", w3_hbm, w3_v), ("w4", w4_hbm, w4_v), ("gw", gw_hbm, gw_ref)]):
            wcp[nm] = pltpu.make_async_copy(src, dst, wsem.at[i])
        wcp["gw"].start()
        xa_cp(-1).start()
        wname = dict(h="w1", k="wk")
        for nm in first_order:
            if nm in wname:
                wcp[wname[nm]].start()
        if w2loop:
            wcp["w2"].start()
        if wqloop:
            wcp["wq"].start()
        for t in range(N1):
            xa_cp(t).start()
        for nm in ["wv", "wo", "wq", "w2", "w3", "w4"]:
            if not (wqloop and nm == "wq") and not (w2loop and nm == "w2"):
                wcp[nm].start()

        if strided:
            h_v[pl.ds(0, HP * NJ), :] = jnp.zeros((HP * NJ, LANE), F32)
            h_v[pl.ds((HP + S) * NJ, 8 * NJ), :] = jnp.zeros((8 * NJ, LANE), F32)
        else:
            h_v[pl.ds(0, HP), :] = jnp.zeros((HP, D), F32)
            h_v[pl.ds(HP + S, 8), :] = jnp.zeros((8, D), F32)

        def store_h(r, n, h):
            if strided:
                for j in range(NJ):
                    h_v[pl.ds((HP + r) * NJ + j, n, stride=NJ), :] = h[:, j * LANE:(j + 1) * LANE]
            else:
                h_v[pl.ds(HP + r, n), :] = h

        def shifted(r, n):
            if strided:
                lane = jax.lax.broadcasted_iota(jnp.int32, (n, LANE), 1)
                def sh(k, j):
                    return h_v[pl.ds((HP + r + k) * NJ + j, n, stride=NJ), :]
                return jnp.concatenate([
                    sh(-1, 0),
                    jnp.where(lane < 32, sh(-1, 1), sh(1, 1)),
                    jnp.where(lane < 64, sh(1, 2), sh(-2, 2)),
                    jnp.where(lane < 96, sh(-2, 3), sh(2, 3)),
                    sh(2, 4)], axis=1)
            w = h_v[pl.ds(HP + r - 8, n + 16), :]
            lane = jax.lax.broadcasted_iota(jnp.int32, (n, LANE), 1)
            cache = {}
            def sh(k, j):
                if (k, j) not in cache:
                    cache[(k, j)] = pltpu.roll(w[:, j * LANE:(j + 1) * LANE], (-k) % (n + 16), 0)[8:8 + n]
                return cache[(k, j)]
            return jnp.concatenate([
                sh(-1, 0),
                jnp.where(lane < 32, sh(-1, 1), sh(1, 1)),
                jnp.where(lane < 64, sh(1, 2), sh(-2, 2)),
                jnp.where(lane < 96, sh(-2, 3), sh(2, 3)),
                sh(2, 4)], axis=1)

        def gate(xf):
            gw = gw_ref[...].astype(F32)
            acc = xf[:, 0:LANE] * gw[0:1, :]
            for j in range(1, NJ):
                acc = acc + xf[:, j * LANE:(j + 1) * LANE] * gw[j:j + 1, :]
            return _sigmoid(jnp.sum(acc, axis=-1, keepdims=True))

        def phase1(t):
            first = isinstance(t, int) and t < 0
            T = T0 if first else T1
            r0 = 0 if first else pl.multiple_of(T0 + t * T1, LANE)
            xa_cp(t).wait()
            if first:
                wcp["gw"].wait()
            xa = xa_v[pl.ds(r0, T), :]
            st = {}
            def mm(a, b):
                if first:
                    hh = T // ms
                    return jnp.concatenate([_dot(a[i * hh:(i + 1) * hh], b) for i in range(ms)], axis=0)
                return _dot(a, b)
            def f_k():
                if first:
                    wcp["wk"].wait()
                    if defer_h0:
                        store_h(r0, T, _gelu(hpre_v[...]))
                pk = _phi(mm(xa, wk_v[...]))
                zs = jnp.sum(pk.reshape(T // 8, 8, D), axis=0)
                if first:
                    z_acc[...] = zs
                else:
                    z_acc[...] += zs
                st["pkt"] = pk.astype(BF).T
            def f_h():
                xf = xa.astype(F32)
                m = jnp.sum(_lane_tiles_sum(xf), axis=-1, keepdims=True) * (1.0 / D)
                xc = xf - m
                v = jnp.sum(_lane_tiles_sum(xc * xc), axis=-1, keepdims=True) * (1.0 / D)
                rs = jax.lax.rsqrt(v + 1e-5)
                ln = (xf * rs - m * rs).astype(BF)
                if gate1:
                    g_v[pl.ds(r0, T), :] = jnp.broadcast_to(gate(xf), (T, LANE))
                mx_v[pl.ds(r0, T), :] = jnp.broadcast_to(m, (T, LANE))
                if first:
                    wcp["w1"].wait()
                if first and defer_h0:
                    hpre_v[...] = mm(ln, w1_v[...])
                    return
                store_h(r0, T, _gelu(mm(ln, w1_v[...])))
            def f_g():
                ns = gs if first else gsl
                hh = D // ns
                gg = jnp.concatenate([_dot(st["pkt"][i * hh:(i + 1) * hh], xa) for i in range(ns)], axis=0)
                if first:
                    g_acc[...] = gg
                else:
                    g_acc[...] += gg
            fs = dict(k=f_k, h=f_h, g=f_g)
            for nm in (first_order if first else order1):
                fs[nm]()

        phase1(-1)
        def body1(t, c):
            phase1(t)
            if w2loop:
                cb2 = pl.multiple_of(jnp.minimum(t, NJ - 1) * LANE, LANE)
                blk = _lane_tiles_sum(w2_v[pl.ds(cb2, LANE), :].astype(F32))
                w2rs_v[:, pl.ds(cb2, LANE)] = jnp.sum(blk.T.reshape(LANE // 8, 8, LANE), axis=0)
            if wqloop:
                cb = pl.multiple_of(jnp.minimum(t, NJ - 1) * LANE, LANE)
                wqt_v[pl.ds(cb, LANE), :] = wq_v[:, pl.ds(cb, LANE)].T
            return c
        if wqloop:
            wcp["wq"].wait()
        if w2loop:
            wcp["w2"].wait()
        jax.lax.fori_loop(0, N1, body1, 0)

        for nm in ["wv", "wo", "wq", "w2", "w3", "w4"]:
            if not (wqloop and nm == "wq") and not (w2loop and nm == "w2"):
                wcp[nm].wait()
        if zbv == 1:
            z = jnp.sum(z_acc[...], axis=0, keepdims=True)
            zb_v[...] = jnp.broadcast_to(z, (LANE, D)).T
        if zbv == 2:
            zt = jnp.sum(z_acc[...].T, axis=1, keepdims=True)
            zb_v[...] = jnp.broadcast_to(zt, (D, LANE))
        if not wqloop:
            wqt_v[...] = wq_v[...].T
        kvms = []
        for j, (lo, hi) in enumerate(BANDS):
            n = hi - lo
            rr = jax.lax.broadcasted_iota(jnp.int32, (n, LANE), 0) + lo
            cc = jax.lax.broadcasted_iota(jnp.int32, (n, LANE), 1) + j * LANE
            kv = _dot(g_acc[pl.ds(lo, n), :].astype(BF), wv_v[:, pl.ds(j * LANE, LANE)])
            kvms.append(jnp.where(_head_of(rr) == _head_of(cc), kv, 0.0).astype(BF))
        parts = [_dot(kvms[j], wo_v[pl.ds(j * LANE, LANE), :]) for j in range(NJ)]
        edges = sorted(set([lo for lo, hi in BANDS] + [hi for lo, hi in BANDS]))
        for a, b in zip(edges[:-1], edges[1:]):
            acc = None
            for j, (lo, hi) in enumerate(BANDS):
                if lo <= a and b <= hi:
                    p = parts[j][a - lo:b - lo]
                    acc = p if acc is None else acc + p
            m_v[pl.ds(a, b - a), :] = acc.astype(BF)
        if not w2loop:
            w2rs_v[...] = _dot_nt(jnp.ones((16, D), BF), w2_v[...])
        if zbv == 0:
            z = jnp.sum(z_acc[...], axis=0, keepdims=True)
            zb_v[...] = jnp.broadcast_to(z, (LANE, D)).T

        OR = min(orows, T2)
        OC = [(c * LANE, 0, T2) for c in range(NJ - 1)] + [((NJ - 1) * LANE, rr, OR) for rr in range(0, T2, OR)]
        def out_cp(t, c):
            c0, rr, nr = OC[c]
            return pltpu.make_async_copy(obuf.at[pl.ds(t * T2 + rr, nr), pl.ds(c0, LANE)],
                                         out_hbm.at[pl.ds(t * T2 + rr, nr), pl.ds(c0, LANE)], osem.at[t * len(OC) + c])

        NP = H // 2
        sub = jax.lax.broadcasted_iota(jnp.int32, (NP, 8, T2), 1)

        def phase2(t, carry):
            r0 = pl.multiple_of(t * T2, T2)
            xa = xa_v[pl.ds(r0, T2), :]
            st = {}
            def f_q():
                st["q"] = _dot_nt(wqt_v[...], xa)
            def f_w2():
                hsb = shifted(r0, T2).astype(BF)
                wr = jnp.sum(w2rs_v[...], axis=0, keepdims=True) if w2loop else w2rs_v[0:1, :]
                u = jnp.sum(_lane_tiles_sum(hsb.astype(F32) * wr), axis=-1, keepdims=True) * (1.0 / D)
                m = mx_v[pl.ds(r0, T2), :] + u
                st["m"] = m
                m5 = jnp.concatenate([m] * NJ, axis=1)
                st["xc"] = (xa.astype(F32) - m5) + _dot(hsb, w2_v[...])
            def f_phi():
                pq = _phi(st["q"])
                zb = zb_v[...]
                tz = pq * jnp.concatenate([zb] * (T2 // LANE), axis=1)
                t4 = tz.reshape(NP, 5, 8, T2)
                p4 = pq.reshape(NP, 5, 8, T2)
                lo4 = sub < 4
                sa = t4[:, 0] + t4[:, 1] + jnp.where(lo4, t4[:, 2], 0.0)
                sb = t4[:, 3] + t4[:, 4] + jnp.where(lo4, 0.0, t4[:, 2])
                def allsum(a):
                    a = a + pltpu.roll(a, 4, 1)
                    a = a + pltpu.roll(a, 2, 1)
                    a = a + pltpu.roll(a, 1, 1)
                    return a
                da = allsum(sa) + 1e-6
                db = allsum(sb) + 1e-6
                def rc(d):
                    r = pl.reciprocal(d, approx=True)
                    return r * (2.0 - d * r)
                ra = rc(da); rb = rc(db)
                pn = jnp.stack([p4[:, 0] * ra, p4[:, 1] * ra, p4[:, 2] * jnp.where(lo4, ra, rb), p4[:, 3] * rb, p4[:, 4] * rb], axis=1)
                st["pqn"] = pn.reshape(D, T2).astype(BF)
            def f_ln():
                xc = st["xc"]
                st["ln"] = xc.astype(BF)
                st["rs"] = jax.lax.rsqrt(jnp.sum(_lane_tiles_sum(xc * xc), axis=-1, keepdims=True) * (1.0 / D) + 1e-5)
            def f_w3():
                h3l = _gelu(_dot_nt(w3_v[FM:F, :], st["ln"]).T * st["rs"]).astype(BF)
                h3m = _gelu(_dot_nt(st["ln"], w3_v[0:FM, :]) * st["rs"]).astype(BF)
                st["h3"] = jnp.concatenate([h3m, h3l], axis=1)
            def f_a():
                st["a"] = _dot_tn(st["pqn"], m_v[...])
            def f_w4():
                st["bm"] = st["xc"] + _dot(st["h3"], w4_v[...])
            fs = dict(q=f_q, w2=f_w2, phi=f_phi, ln=f_ln, w3=f_w3, a=f_a, w4=f_w4)
            for nm in order2:
                fs[nm]()
            g = g_v[pl.ds(r0, T2), :] if gate1 else jnp.broadcast_to(gate(xa.astype(F32)), (T2, LANE))
            for c, (c0, rr, nr) in enumerate(OC):
                b = st["bm"][rr:rr + nr, c0:c0 + LANE] + st["m"][rr:rr + nr]
                obuf[pl.ds(r0 + rr, nr), pl.ds(c0, LANE)] = (b + g[rr:rr + nr] * (st["a"][rr:rr + nr, c0:c0 + LANE] - b)).astype(BF)
                out_cp(t, c).start()
            return carry
        jax.lax.fori_loop(0, N2, phase2, 0)
        for t in range(N2):
            for c in range(len(OC)):
                out_cp(t, c).wait()

    @jax.jit
    def fn(A_x, A_wqkv, A_wo, B_x, B_w1, B_w2, B_w3, B_w4, gate_w):
        any_spec = pl.BlockSpec(memory_space=pltpu.HBM)
        out = pl.pallas_call(
            kernel,
            out_shape=jax.ShapeDtypeStruct((S, D), BF),
            in_specs=[any_spec] * 8,
            out_specs=any_spec,
            scratch_shapes=[
                pltpu.VMEM((S, D), BF),
                pltpu.VMEM((D, D), BF), pltpu.VMEM((D, D), BF), pltpu.VMEM((D, D), BF),
                pltpu.VMEM((D, D), BF), pltpu.VMEM((D, D), BF), pltpu.VMEM((D, D), BF),
                pltpu.VMEM((F, D), BF), pltpu.VMEM((F, D), BF),
                pltpu.VMEM((NJ, LANE), BF), pltpu.VMEM((T0, D), F32), pltpu.VMEM((8 if w2loop else 16, D), F32),
                pltpu.VMEM(((HP + S + 8) * NJ, LANE) if strided else (HP + S + 8, D), F32),
                pltpu.VMEM((S, LANE), F32), pltpu.VMEM((S, LANE), F32),
                pltpu.VMEM((D, D), BF),
                pltpu.VMEM((D, D), F32), pltpu.VMEM((8, D), F32),
                pltpu.VMEM((D, D), BF), pltpu.VMEM((D, LANE), F32),
                pltpu.VMEM((S, D), BF),
                pltpu.SemaphoreType.DMA((NW + 1 + N1,)),
                pltpu.SemaphoreType.DMA((N2 * (NJ - 1 + T2 // min(orows, T2)),)),
            ],
            compiler_params=pltpu.CompilerParams(vmem_limit_bytes=100 * 1024 * 1024),
            name="gmix",
        )(A_x.reshape(S, D), A_wqkv, A_wo, B_w1, B_w2, B_w3.T, B_w4, gate_w.reshape(NJ, LANE))
        return out.reshape(1, S, D)
    return fn


pallas_gated_mix__linear_attn_block__mixer_s_mlp__prompt_kernel = make()
```

```python
import jax
import jax.numpy as jnp
import jax.experimental.pallas as pl
import jax.experimental.pallas.tpu as pltpu

S, D, F, H, DH = 2048, 640, 1728, 32, 20
LANE = 128
NJ = D // LANE
FM = (F // LANE) * LANE
BF = jnp.bfloat16
F32 = jnp.float32
HP = 8


def _bands():
    out = []
    for j in range(NJ):
        h_lo = (LANE * j) // DH
        h_hi = (LANE * (j + 1) - 1) // DH
        lo = (h_lo * DH) // 16 * 16
        hi = -(-((h_hi + 1) * DH) // 16) * 16
        out.append((lo, hi))
    return out
BANDS = _bands()


def _head_of(idx):
    return (idx * 3277) >> 16


def _gelu(x):
    c = 0.7978845608028654
    hx = 0.5 * x
    u = x * (c + (c * 0.044715) * (x * x))
    return hx + hx * jnp.tanh(u)


def _phi(t):
    return jnp.where(t > 0, t + 1.0, jnp.exp(t)) + 1e-6


def _sigmoid(x):
    return 0.5 + 0.5 * jnp.tanh(0.5 * x)


def _dot(a, b):
    return jnp.dot(a, b, preferred_element_type=F32)


def _dot_nt(a, b):
    return jax.lax.dot_general(a, b, (((1,), (1,)), ((), ())), preferred_element_type=F32)


def _dot_tn(a, b):
    return jax.lax.dot_general(a, b, (((0,), (0,)), ((), ())), preferred_element_type=F32)


def _lane_tiles_sum(x):
    acc = x[:, 0:LANE]
    for j in range(1, x.shape[1] // LANE):
        acc = acc + x[:, j * LANE:(j + 1) * LANE]
    return acc


def make(T0=256, T1=256, T2=1024, order2="q,phi,w2,ln,a,w3,w4", order1="k,h,g", first_order="h,k,g", orows=128, strided=True, gate1=True, defer_h0=False, ms=4, gs=2, gsl=1, zbv=1, wqloop=False, w2loop=True, gwpos=0, cparams=None):
    N1 = (S - T0) // T1
    assert T0 + N1 * T1 == S
    N2 = S // T2
    order2 = order2.split(",")
    order1 = order1.split(",")
    first_order = first_order.split(",")
    NW = 9

    def kernel(xa_hbm, wqkv_hbm, wo_hbm, w1_hbm, w2_hbm, w3_hbm, w4_hbm, gw_hbm,
               out_hbm,
               xa_v, wq_v, wk_v, wv_v, wo_v, w1_v, w2_v, w3_v, w4_v,
               gw_ref, hpre_v, w2rs_v, h_v, g_v, mx_v, wqt_v, g_acc, z_acc, m_v, zb_v, obuf,
               wsem, osem):
        def xa_cp(t):
            if isinstance(t, int) and t < 0:
                return pltpu.make_async_copy(xa_hbm.at[pl.ds(0, T0)], xa_v.at[pl.ds(0, T0)], wsem.at[NW])
            return pltpu.make_async_copy(xa_hbm.at[pl.ds(T0 + t * T1, T1)], xa_v.at[pl.ds(T0 + t * T1, T1)], wsem.at[NW + 1 + t])
        wcp = {}
        for i, (nm, src, dst) in enumerate([
                ("wq", wqkv_hbm.at[:, pl.ds(0, D)], wq_v), ("wk", wqkv_hbm.at[:, pl.ds(D, D)], wk_v),
                ("wv", wqkv_hbm.at[:, pl.ds(2 * D, D)], wv_v),
                ("w1", w1_hbm, w1_v), ("wo", wo_hbm, wo_v),
                ("w2", w2_hbm, w2_v), ("w3", w3_hbm, w3_v), ("w4", w4_hbm, w4_v), ("gw", gw_hbm, gw_ref)]):
            wcp[nm] = pltpu.make_async_copy(src, dst, wsem.at[i])
        if gwpos == 0:
            wcp["gw"].start()
        xa_cp(-1).start()
        if gwpos == 1:
            wcp["gw"].start()
        wname = dict(h="w1", k="wk")
        for nm in first_order:
            if nm in wname:
                wcp[wname[nm]].start()
        if w2loop:
            wcp["w2"].start()
        if wqloop:
            wcp["wq"].start()
        for t in range(N1):
            xa_cp(t).start()
        for nm in ["wv", "wo", "wq", "w2", "w3", "w4"]:
            if not (wqloop and nm == "wq") and not (w2loop and nm == "w2"):
                wcp[nm].start()

        if strided:
            h_v[pl.ds(0, HP * NJ), :] = jnp.zeros((HP * NJ, LANE), F32)
            h_v[pl.ds((HP + S) * NJ, 8 * NJ), :] = jnp.zeros((8 * NJ, LANE), F32)
        else:
            h_v[pl.ds(0, HP), :] = jnp.zeros((HP, D), F32)
            h_v[pl.ds(HP + S, 8), :] = jnp.zeros((8, D), F32)

        def store_h(r, n, h):
            if strided:
                for j in range(NJ):
                    h_v[pl.ds((HP + r) * NJ + j, n, stride=NJ), :] = h[:, j * LANE:(j + 1) * LANE]
            else:
                h_v[pl.ds(HP + r, n), :] = h

        def shifted(r, n):
            if strided:
                lane = jax.lax.broadcasted_iota(jnp.int32, (n, LANE), 1)
                def sh(k, j):
                    return h_v[pl.ds((HP + r + k) * NJ + j, n, stride=NJ), :]
                return jnp.concatenate([
                    sh(-1, 0),
                    jnp.where(lane < 32, sh(-1, 1), sh(1, 1)),
                    jnp.where(lane < 64, sh(1, 2), sh(-2, 2)),
                    jnp.where(lane < 96, sh(-2, 3), sh(2, 3)),
                    sh(2, 4)], axis=1)
            w = h_v[pl.ds(HP + r - 8, n + 16), :]
            lane = jax.lax.broadcasted_iota(jnp.int32, (n, LANE), 1)
            cache = {}
            def sh(k, j):
                if (k, j) not in cache:
                    cache[(k, j)] = pltpu.roll(w[:, j * LANE:(j + 1) * LANE], (-k) % (n + 16), 0)[8:8 + n]
                return cache[(k, j)]
            return jnp.concatenate([
                sh(-1, 0),
                jnp.where(lane < 32, sh(-1, 1), sh(1, 1)),
                jnp.where(lane < 64, sh(1, 2), sh(-2, 2)),
                jnp.where(lane < 96, sh(-2, 3), sh(2, 3)),
                sh(2, 4)], axis=1)

        def gate(xf):
            gw = gw_ref[...].astype(F32)
            acc = xf[:, 0:LANE] * gw[0:1, :]
            for j in range(1, NJ):
                acc = acc + xf[:, j * LANE:(j + 1) * LANE] * gw[j:j + 1, :]
            return _sigmoid(jnp.sum(acc, axis=-1, keepdims=True))

        def phase1(t):
            first = isinstance(t, int) and t < 0
            T = T0 if first else T1
            r0 = 0 if first else pl.multiple_of(T0 + t * T1, LANE)
            xa_cp(t).wait()
            if first:
                wcp["gw"].wait()
            xa = xa_v[pl.ds(r0, T), :]
            st = {}
            def mm(a, b):
                if first:
                    hh = T // ms
                    return jnp.concatenate([_dot(a[i * hh:(i + 1) * hh], b) for i in range(ms)], axis=0)
                return _dot(a, b)
            def f_k():
                if first:
                    wcp["wk"].wait()
                    if defer_h0:
                        store_h(r0, T, _gelu(hpre_v[...]))
                pk = _phi(mm(xa, wk_v[...]))
                zs = jnp.sum(pk.reshape(T // 8, 8, D), axis=0)
                if first:
                    z_acc[...] = zs
                else:
                    z_acc[...] += zs
                st["pkt"] = pk.astype(BF).T
            def f_h():
                xf = xa.astype(F32)
                m = jnp.sum(_lane_tiles_sum(xf), axis=-1, keepdims=True) * (1.0 / D)
                xc = xf - m
                v = jnp.sum(_lane_tiles_sum(xc * xc), axis=-1, keepdims=True) * (1.0 / D)
                rs = jax.lax.rsqrt(v + 1e-5)
                ln = (xf * rs - m * rs).astype(BF)
                if gate1:
                    g_v[pl.ds(r0, T), :] = jnp.broadcast_to(gate(xf), (T, LANE))
                mx_v[pl.ds(r0, T), :] = jnp.broadcast_to(m, (T, LANE))
                if first:
                    wcp["w1"].wait()
                if first and defer_h0:
                    hpre_v[...] = mm(ln, w1_v[...])
                    return
                store_h(r0, T, _gelu(mm(ln, w1_v[...])))
            def f_g():
                ns = gs if first else gsl
                hh = D // ns
                gg = jnp.concatenate([_dot(st["pkt"][i * hh:(i + 1) * hh], xa) for i in range(ns)], axis=0)
                if first:
                    g_acc[...] = gg
                else:
                    g_acc[...] += gg
            fs = dict(k=f_k, h=f_h, g=f_g)
            for nm in (first_order if first else order1):
                fs[nm]()

        phase1(-1)
        def body1(t, c):
            phase1(t)
            if w2loop:
                cb2 = pl.multiple_of(jnp.minimum(t, NJ - 1) * LANE, LANE)
                blk = _lane_tiles_sum(w2_v[pl.ds(cb2, LANE), :].astype(F32))
                w2rs_v[:, pl.ds(cb2, LANE)] = jnp.sum(blk.T.reshape(LANE // 8, 8, LANE), axis=0)
            if wqloop:
                cb = pl.multiple_of(jnp.minimum(t, NJ - 1) * LANE, LANE)
                wqt_v[pl.ds(cb, LANE), :] = wq_v[:, pl.ds(cb, LANE)].T
            return c
        if wqloop:
            wcp["wq"].wait()
        if w2loop:
            wcp["w2"].wait()
        jax.lax.fori_loop(0, N1, body1, 0)

        for nm in ["wv", "wo", "wq", "w2", "w3", "w4"]:
            if not (wqloop and nm == "wq") and not (w2loop and nm == "w2"):
                wcp[nm].wait()
        if zbv == 1:
            z = jnp.sum(z_acc[...], axis=0, keepdims=True)
            zb_v[...] = jnp.broadcast_to(z, (LANE, D)).T
        if zbv == 2:
            zt = jnp.sum(z_acc[...].T, axis=1, keepdims=True)
            zb_v[...] = jnp.broadcast_to(zt, (D, LANE))
        if not wqloop:
            wqt_v[...] = wq_v[...].T
        kvms = []
        for j, (lo, hi) in enumerate(BANDS):
            n = hi - lo
            rr = jax.lax.broadcasted_iota(jnp.int32, (n, LANE), 0) + lo
            cc = jax.lax.broadcasted_iota(jnp.int32, (n, LANE), 1) + j * LANE
            kv = _dot(g_acc[pl.ds(lo, n), :].astype(BF), wv_v[:, pl.ds(j * LANE, LANE)])
            kvms.append(jnp.where(_head_of(rr) == _head_of(cc), kv, 0.0).astype(BF))
        parts = [_dot(kvms[j], wo_v[pl.ds(j * LANE, LANE), :]) for j in range(NJ)]
        edges = sorted(set([lo for lo, hi in BANDS] + [hi for lo, hi in BANDS]))
        for a, b in zip(edges[:-1], edges[1:]):
            acc = None
            for j, (lo, hi) in enumerate(BANDS):
                if lo <= a and b <= hi:
                    p = parts[j][a - lo:b - lo]
                    acc = p if acc is None else acc + p
            m_v[pl.ds(a, b - a), :] = acc.astype(BF)
        if not w2loop:
            w2rs_v[...] = _dot_nt(jnp.ones((16, D), BF), w2_v[...])
        if zbv == 0:
            z = jnp.sum(z_acc[...], axis=0, keepdims=True)
            zb_v[...] = jnp.broadcast_to(z, (LANE, D)).T

        OR = min(orows, T2)
        OC = [(c * LANE, 0, T2) for c in range(NJ - 1)] + [((NJ - 1) * LANE, rr, OR) for rr in range(0, T2, OR)]
        def out_cp(t, c):
            c0, rr, nr = OC[c]
            return pltpu.make_async_copy(obuf.at[pl.ds(t * T2 + rr, nr), pl.ds(c0, LANE)],
                                         out_hbm.at[pl.ds(t * T2 + rr, nr), pl.ds(c0, LANE)], osem.at[0])

        NP = H // 2
        sub = jax.lax.broadcasted_iota(jnp.int32, (NP, 8, T2), 1)

        def phase2(t, carry):
            r0 = pl.multiple_of(t * T2, T2)
            xa = xa_v[pl.ds(r0, T2), :]
            st = {}
            def f_q():
                st["q"] = _dot_nt(wqt_v[...], xa)
            def f_w2():
                hsb = shifted(r0, T2).astype(BF)
                wr = jnp.sum(w2rs_v[...], axis=0, keepdims=True) if w2loop else w2rs_v[0:1, :]
                u = jnp.sum(_lane_tiles_sum(hsb.astype(F32) * wr), axis=-1, keepdims=True) * (1.0 / D)
                m = mx_v[pl.ds(r0, T2), :] + u
                st["m"] = m
                m5 = jnp.concatenate([m] * NJ, axis=1)
                st["xc"] = (xa.astype(F32) - m5) + _dot(hsb, w2_v[...])
            def f_phi():
                pq = _phi(st["q"])
                zb = zb_v[...]
                tz = pq * jnp.concatenate([zb] * (T2 // LANE), axis=1)
                t4 = tz.reshape(NP, 5, 8, T2)
                p4 = pq.reshape(NP, 5, 8, T2)
                lo4 = sub < 4
                sa = t4[:, 0] + t4[:, 1] + jnp.where(lo4, t4[:, 2], 0.0)
                sb = t4[:, 3] + t4[:, 4] + jnp.where(lo4, 0.0, t4[:, 2])
                def allsum(a):
                    a = a + pltpu.roll(a, 4, 1)
                    a = a + pltpu.roll(a, 2, 1)
                    a = a + pltpu.roll(a, 1, 1)
                    return a
                da = allsum(sa) + 1e-6
                db = allsum(sb) + 1e-6
                def rc(d):
                    r = pl.reciprocal(d, approx=True)
                    return r * (2.0 - d * r)
                ra = rc(da); rb = rc(db)
                pn = jnp.stack([p4[:, 0] * ra, p4[:, 1] * ra, p4[:, 2] * jnp.where(lo4, ra, rb), p4[:, 3] * rb, p4[:, 4] * rb], axis=1)
                st["pqn"] = pn.reshape(D, T2).astype(BF)
            def f_ln():
                xc = st["xc"]
                st["ln"] = xc.astype(BF)
                st["rs"] = jax.lax.rsqrt(jnp.sum(_lane_tiles_sum(xc * xc), axis=-1, keepdims=True) * (1.0 / D) + 1e-5)
            def f_w3():
                h3l = _gelu(_dot_nt(w3_v[FM:F, :], st["ln"]).T * st["rs"]).astype(BF)
                h3m = _gelu(_dot_nt(st["ln"], w3_v[0:FM, :]) * st["rs"]).astype(BF)
                st["h3"] = jnp.concatenate([h3m, h3l], axis=1)
            def f_a():
                st["a"] = _dot_tn(st["pqn"], m_v[...])
            def f_w4():
                st["bm"] = st["xc"] + _dot(st["h3"], w4_v[...])
            fs = dict(q=f_q, w2=f_w2, phi=f_phi, ln=f_ln, w3=f_w3, a=f_a, w4=f_w4)
            for nm in order2:
                fs[nm]()
            g = g_v[pl.ds(r0, T2), :] if gate1 else jnp.broadcast_to(gate(xa.astype(F32)), (T2, LANE))
            for c, (c0, rr, nr) in enumerate(OC):
                b = st["bm"][rr:rr + nr, c0:c0 + LANE] + st["m"][rr:rr + nr]
                obuf[pl.ds(r0 + rr, nr), pl.ds(c0, LANE)] = (b + g[rr:rr + nr] * (st["a"][rr:rr + nr, c0:c0 + LANE] - b)).astype(BF)
                out_cp(t, c).start()
            return carry
        jax.lax.fori_loop(0, N2, phase2, 0)
        pltpu.make_async_copy(obuf, out_hbm, osem.at[0]).wait()

    @jax.jit
    def fn(A_x, A_wqkv, A_wo, B_x, B_w1, B_w2, B_w3, B_w4, gate_w):
        any_spec = pl.BlockSpec(memory_space=pltpu.HBM)
        out = pl.pallas_call(
            kernel,
            out_shape=jax.ShapeDtypeStruct((S, D), BF),
            in_specs=[any_spec] * 8,
            out_specs=any_spec,
            scratch_shapes=[
                pltpu.VMEM((S, D), BF),
                pltpu.VMEM((D, D), BF), pltpu.VMEM((D, D), BF), pltpu.VMEM((D, D), BF),
                pltpu.VMEM((D, D), BF), pltpu.VMEM((D, D), BF), pltpu.VMEM((D, D), BF),
                pltpu.VMEM((F, D), BF), pltpu.VMEM((F, D), BF),
                pltpu.VMEM((NJ, LANE), BF), pltpu.VMEM((T0, D), F32), pltpu.VMEM((8 if w2loop else 16, D), F32),
                pltpu.VMEM(((HP + S + 8) * NJ, LANE) if strided else (HP + S + 8, D), F32),
                pltpu.VMEM((S, LANE), F32), pltpu.VMEM((S, LANE), F32),
                pltpu.VMEM((D, D), BF),
                pltpu.VMEM((D, D), F32), pltpu.VMEM((8, D), F32),
                pltpu.VMEM((D, D), BF), pltpu.VMEM((D, LANE), F32),
                pltpu.VMEM((S, D), BF),
                pltpu.SemaphoreType.DMA((NW + 1 + N1,)),
                pltpu.SemaphoreType.DMA((1,)),
            ],
            compiler_params=pltpu.CompilerParams(vmem_limit_bytes=100 * 1024 * 1024, disable_bounds_checks=True, disable_semaphore_checks=True, **(cparams or {})),
            name="gmix",
        )(A_x.reshape(S, D), A_wqkv, A_wo, B_w1, B_w2, B_w3.T, B_w4, gate_w.reshape(NJ, LANE))
        return out.reshape(1, S, D)
    return fn


pallas_gated_mix__linear_attn_block__mixer_s_mlp__prompt_kernel = make()
```

```python
import jax
import jax.numpy as jnp
import jax.experimental.pallas as pl
import jax.experimental.pallas.tpu as pltpu

S, D, F, H, DH = 2048, 640, 1728, 32, 20
LANE = 128
NJ = D // LANE
FM = (F // LANE) * LANE
BF = jnp.bfloat16
F32 = jnp.float32

T0 = 256
T1 = 256
N1 = (S - T0) // T1
T2 = 1024
N2 = S // T2
HP = 8
KS = 256
OR = 128
NW = 10


def _bands():
    out = []
    for j in range(NJ):
        h_lo = (LANE * j) // DH
        h_hi = (LANE * (j + 1) - 1) // DH
        out.append(((h_lo * DH) // 16 * 16, -(-((h_hi + 1) * DH) // 16) * 16))
    return out


BANDS = _bands()


def _head_of(idx):
    return (idx * 3277) >> 16


def _gelu(x):
    c = 0.7978845608028654
    hx = 0.5 * x
    u = x * (c + (c * 0.044715) * (x * x))
    return hx + hx * jnp.tanh(u)


def _phi(t):
    return jnp.where(t > 0, t + 1.0, jnp.exp(t)) + 1e-6


def _sigmoid(x):
    return 0.5 + 0.5 * jnp.tanh(0.5 * x)


def _dot(a, b):
    return jnp.dot(a, b, preferred_element_type=F32)


def _dot_nt(a, b):
    return jax.lax.dot_general(a, b, (((1,), (1,)), ((), ())), preferred_element_type=F32)


def _dot_tn(a, b):
    return jax.lax.dot_general(a, b, (((0,), (0,)), ((), ())), preferred_element_type=F32)


def _dot_rows(a, b, n):
    r = a.shape[0] // n
    return jnp.concatenate([_dot(a[i * r:(i + 1) * r], b) for i in range(n)], axis=0)


def _lane_tiles_sum(x):
    acc = x[:, 0:LANE]
    for j in range(1, x.shape[1] // LANE):
        acc = acc + x[:, j * LANE:(j + 1) * LANE]
    return acc


def _row_mean(x):
    return jnp.sum(_lane_tiles_sum(x), axis=-1, keepdims=True) * (1.0 / D)


def _kernel(x_hbm, wqkv_hbm, wo_hbm, w1_hbm, w2_hbm, w3_hbm, w4_hbm, gw_hbm,
            out_hbm,
            x_v, wq_v, wk_v, wv_v, wo_v, w1_v, w2_v, w3_v, w4_v, gw_v,
            w2rs_v, h_v, g_v, mx_v, wqt_v, g_acc, z_acc, m_v, zb_v, obuf,
            isem, osem):
    def x_cp(t):
        if isinstance(t, int) and t < 0:
            return pltpu.make_async_copy(x_hbm.at[pl.ds(0, T0)], x_v.at[pl.ds(0, T0)], isem.at[NW])
        return pltpu.make_async_copy(x_hbm.at[pl.ds(T0 + t * T1, T1)], x_v.at[pl.ds(T0 + t * T1, T1)],
                                     isem.at[NW + 1 + t])

    srcs = [
        ("gw", gw_hbm, gw_v),
        ("wka", wqkv_hbm.at[pl.ds(0, KS), pl.ds(D, D)], wk_v.at[pl.ds(0, KS)]),
        ("wkb", wqkv_hbm.at[pl.ds(KS, D - KS), pl.ds(D, D)], wk_v.at[pl.ds(KS, D - KS)]),
        ("w1", w1_hbm, w1_v), ("w2", w2_hbm, w2_v),
        ("wv", wqkv_hbm.at[:, pl.ds(2 * D, D)], wv_v), ("wo", wo_hbm, wo_v),
        ("wq", wqkv_hbm.at[:, pl.ds(0, D)], wq_v), ("w3", w3_hbm, w3_v), ("w4", w4_hbm, w4_v),
    ]
    wcp = {nm: pltpu.make_async_copy(src, dst, isem.at[i]) for i, (nm, src, dst) in enumerate(srcs)}
    wcp["gw"].start()
    x_cp(-1).start()
    for nm in ("wka", "wkb", "w1", "w2"):
        wcp[nm].start()
    for t in range(N1):
        x_cp(t).start()
    for nm in ("wv", "wo", "wq", "w3", "w4"):
        wcp[nm].start()

    h_v[pl.ds(0, HP * NJ), :] = jnp.zeros((HP * NJ, LANE), F32)
    h_v[pl.ds((HP + S) * NJ, HP * NJ), :] = jnp.zeros((HP * NJ, LANE), F32)

    def store_h(r, n, h):
        for j in range(NJ):
            h_v[pl.ds((HP + r) * NJ + j, n, stride=NJ), :] = h[:, j * LANE:(j + 1) * LANE]

    def shifted_h(r, n):
        lane = jax.lax.broadcasted_iota(jnp.int32, (n, LANE), 1)

        def sh(k, j):
            return h_v[pl.ds((HP + r + k) * NJ + j, n, stride=NJ), :]

        return jnp.concatenate([
            sh(-1, 0),
            jnp.where(lane < 32, sh(-1, 1), sh(1, 1)),
            jnp.where(lane < 64, sh(1, 2), sh(-2, 2)),
            jnp.where(lane < 96, sh(-2, 3), sh(2, 3)),
            sh(2, 4)], axis=1)

    def row_stats(r0, n, xb):
        xf = xb.astype(F32)
        m = _row_mean(xf)
        xc = xf - m
        rs = jax.lax.rsqrt(_row_mean(xc * xc) + 1e-5)
        gw = gw_v[...].astype(F32)
        acc = xf[:, 0:LANE] * gw[0:1, :]
        for j in range(1, NJ):
            acc = acc + xf[:, j * LANE:(j + 1) * LANE] * gw[j:j + 1, :]
        gate = _sigmoid(jnp.sum(acc, axis=-1, keepdims=True))
        g_v[pl.ds(r0, n), :] = jnp.broadcast_to(gate, (n, LANE))
        mx_v[pl.ds(r0, n), :] = jnp.broadcast_to(m, (n, LANE))
        return (xf * rs - m * rs).astype(BF)

    def col_sums8(pk):
        return jnp.sum(pk.reshape(pk.shape[0] // 8, 8, D), axis=0)

    x_cp(-1).wait()
    wcp["gw"].wait()
    x0 = x_v[pl.ds(0, T0), :]
    ln0 = row_stats(0, T0, x0)
    wcp["wka"].wait()
    k0 = _dot_rows(x0[:, :KS], wk_v[0:KS, :], 4)
    wcp["wkb"].wait()
    pk0 = _phi(k0 + _dot_rows(x0[:, KS:], wk_v[KS:D, :], 4))
    z_acc[...] = col_sums8(pk0)
    g_acc[...] = _dot_rows(pk0.astype(BF).T, x0, 2)
    wcp["w1"].wait()
    store_h(0, T0, _gelu(_dot_rows(ln0, w1_v[...], 4)))
    wcp["w2"].wait()

    def phase1(t, carry):
        r0 = pl.multiple_of(T0 + t * T1, LANE)
        x_cp(t).wait()
        xb = x_v[pl.ds(r0, T1), :]
        pk = _phi(_dot(xb, wk_v[...]))
        z_acc[...] += col_sums8(pk)
        pkt = pk.astype(BF).T
        ln = row_stats(r0, T1, xb)
        store_h(r0, T1, _gelu(_dot(ln, w1_v[...])))
        g_acc[...] += _dot(pkt, xb)
        cb = pl.multiple_of(jnp.minimum(t, NJ - 1) * LANE, LANE)
        blk = _lane_tiles_sum(w2_v[pl.ds(cb, LANE), :].astype(F32))
        w2rs_v[:, pl.ds(cb, LANE)] = jnp.sum(blk.T.reshape(LANE // 8, 8, LANE), axis=0)
        return carry

    jax.lax.fori_loop(0, N1, phase1, 0)

    for nm in ("wv", "wo", "wq", "w3", "w4"):
        wcp[nm].wait()
    z = jnp.sum(z_acc[...], axis=0, keepdims=True)
    zb_v[...] = jnp.broadcast_to(z, (LANE, D)).T
    wqt_v[...] = wq_v[...].T
    kvm = []
    for j, (lo, hi) in enumerate(BANDS):
        n = hi - lo
        rr = jax.lax.broadcasted_iota(jnp.int32, (n, LANE), 0) + lo
        cc = jax.lax.broadcasted_iota(jnp.int32, (n, LANE), 1) + j * LANE
        kv = _dot(g_acc[pl.ds(lo, n), :].astype(BF), wv_v[:, pl.ds(j * LANE, LANE)])
        kvm.append(jnp.where(_head_of(rr) == _head_of(cc), kv, 0.0).astype(BF))
    parts = [_dot(kvm[j], wo_v[pl.ds(j * LANE, LANE), :]) for j in range(NJ)]
    edges = sorted(set([lo for lo, _ in BANDS] + [hi for _, hi in BANDS]))
    for a, b in zip(edges[:-1], edges[1:]):
        acc = None
        for j, (lo, hi) in enumerate(BANDS):
            if lo <= a and b <= hi:
                p = parts[j][a - lo:b - lo]
                acc = p if acc is None else acc + p
        m_v[pl.ds(a, b - a), :] = acc.astype(BF)

    pieces = [(c * LANE, 0, T2) for c in range(NJ - 1)] + [((NJ - 1) * LANE, r, OR) for r in range(0, T2, OR)]
    NP = H // 2
    lo4 = jax.lax.broadcasted_iota(jnp.int32, (NP, 8, T2), 1) < 4

    def all_sublanes_sum(a):
        a = a + pltpu.roll(a, 4, 1)
        a = a + pltpu.roll(a, 2, 1)
        return a + pltpu.roll(a, 1, 1)

    def recip(d):
        r = pl.reciprocal(d, approx=True)
        return r * (2.0 - d * r)

    def phase2(t, carry):
        r0 = pl.multiple_of(t * T2, T2)
        xb = x_v[pl.ds(r0, T2), :]
        pq = _phi(_dot_nt(wqt_v[...], xb))
        tz = (pq * jnp.concatenate([zb_v[...]] * (T2 // LANE), axis=1)).reshape(NP, 5, 8, T2)
        p4 = pq.reshape(NP, 5, 8, T2)
        ra = recip(all_sublanes_sum(tz[:, 0] + tz[:, 1] + jnp.where(lo4, tz[:, 2], 0.0)) + 1e-6)
        rb = recip(all_sublanes_sum(tz[:, 3] + tz[:, 4] + jnp.where(lo4, 0.0, tz[:, 2])) + 1e-6)
        pqn = jnp.stack([p4[:, 0] * ra, p4[:, 1] * ra, p4[:, 2] * jnp.where(lo4, ra, rb),
                         p4[:, 3] * rb, p4[:, 4] * rb], axis=1).reshape(D, T2).astype(BF)
        hs = shifted_h(r0, T2).astype(BF)
        w2rs = jnp.sum(w2rs_v[...], axis=0, keepdims=True)
        m = mx_v[pl.ds(r0, T2), :] + _row_mean(hs.astype(F32) * w2rs)
        xc = (xb.astype(F32) - jnp.concatenate([m] * NJ, axis=1)) + _dot(hs, w2_v[...])
        ln = xc.astype(BF)
        rs = jax.lax.rsqrt(_row_mean(xc * xc) + 1e-5)
        a = _dot_tn(pqn, m_v[...])
        h3l = _gelu(_dot_nt(w3_v[FM:F, :], ln).T * rs).astype(BF)
        h3m = _gelu(_dot_nt(ln, w3_v[0:FM, :]) * rs).astype(BF)
        bm = xc + _dot(jnp.concatenate([h3m, h3l], axis=1), w4_v[...])
        g = g_v[pl.ds(r0, T2), :]
        for c0, rr, nr in pieces:
            b = bm[rr:rr + nr, c0:c0 + LANE] + m[rr:rr + nr]
            obuf[pl.ds(r0 + rr, nr), pl.ds(c0, LANE)] = (
                b + g[rr:rr + nr] * (a[rr:rr + nr, c0:c0 + LANE] - b)).astype(BF)
            pltpu.make_async_copy(obuf.at[pl.ds(r0 + rr, nr), pl.ds(c0, LANE)],
                                  out_hbm.at[pl.ds(r0 + rr, nr), pl.ds(c0, LANE)], osem.at[0]).start()
        return carry

    jax.lax.fori_loop(0, N2, phase2, 0)
    pltpu.make_async_copy(obuf, out_hbm, osem.at[0]).wait()


@jax.jit
def pallas_gated_mix__linear_attn_block__mixer_s_mlp__prompt_kernel(
        A_x, A_wqkv, A_wo, B_x, B_w1, B_w2, B_w3, B_w4, gate_w):
    del B_x
    hbm = pl.BlockSpec(memory_space=pltpu.HBM)
    out = pl.pallas_call(
        _kernel,
        out_shape=jax.ShapeDtypeStruct((S, D), BF),
        in_specs=[hbm] * 8,
        out_specs=hbm,
        scratch_shapes=[
            pltpu.VMEM((S, D), BF),
            pltpu.VMEM((D, D), BF), pltpu.VMEM((D, D), BF), pltpu.VMEM((D, D), BF),
            pltpu.VMEM((D, D), BF), pltpu.VMEM((D, D), BF), pltpu.VMEM((D, D), BF),
            pltpu.VMEM((F, D), BF), pltpu.VMEM((F, D), BF),
            pltpu.VMEM((NJ, LANE), BF),
            pltpu.VMEM((8, D), F32),
            pltpu.VMEM(((HP + S + HP) * NJ, LANE), F32),
            pltpu.VMEM((S, LANE), F32), pltpu.VMEM((S, LANE), F32),
            pltpu.VMEM((D, D), BF),
            pltpu.VMEM((D, D), F32), pltpu.VMEM((8, D), F32),
            pltpu.VMEM((D, D), BF), pltpu.VMEM((D, LANE), F32),
            pltpu.VMEM((S, D), BF),
            pltpu.SemaphoreType.DMA((NW + 1 + N1,)),
            pltpu.SemaphoreType.DMA((1,)),
        ],
        compiler_params=pltpu.CompilerParams(
            vmem_limit_bytes=100 * 1024 * 1024,
            disable_bounds_checks=True,
            disable_semaphore_checks=True,
        ),
        name="gmix",
    )(A_x.reshape(S, D), A_wqkv, A_wo, B_w1, B_w2, B_w3.T, B_w4, gate_w.reshape(NJ, LANE))
    return out.reshape(1, S, D)
```

```python
import jax
import jax.numpy as jnp
import jax.experimental.pallas as pl
import jax.experimental.pallas.tpu as pltpu

S, D, F, H, DH = 2048, 640, 1728, 32, 20
LANE = 128
NJ = D // LANE
FM = (F // LANE) * LANE
BF = jnp.bfloat16
F32 = jnp.float32

T0 = 256
T1 = 256
N1 = (S - T0) // T1
T2 = 1024
N2 = S // T2
HP = 8
KS = 256
OR = 128
NW = 10


def _bands():
    out = []
    for j in range(NJ):
        h_lo = (LANE * j) // DH
        h_hi = (LANE * (j + 1) - 1) // DH
        out.append(((h_lo * DH) // 16 * 16, -(-((h_hi + 1) * DH) // 16) * 16))
    return out


BANDS = _bands()


def _head_of(idx):
    return (idx * 3277) >> 16


def _gelu(x):
    c = 0.7978845608028654
    hx = 0.5 * x
    u = x * (c + (c * 0.044715) * (x * x))
    return hx + hx * jnp.tanh(u)


def _phi(t):
    return jnp.where(t > 0, t + 1.0, jnp.exp(t)) + 1e-6


def _sigmoid(x):
    return 0.5 + 0.5 * jnp.tanh(0.5 * x)


def _dot(a, b):
    return jnp.dot(a, b, preferred_element_type=F32)


def _dot_nt(a, b):
    return jax.lax.dot_general(a, b, (((1,), (1,)), ((), ())), preferred_element_type=F32)


def _dot_tn(a, b):
    return jax.lax.dot_general(a, b, (((0,), (0,)), ((), ())), preferred_element_type=F32)


def _dot_rows(a, b, n):
    r = a.shape[0] // n
    return jnp.concatenate([_dot(a[i * r:(i + 1) * r], b) for i in range(n)], axis=0)


def _lane_tiles_sum(x):
    acc = x[:, 0:LANE]
    for j in range(1, x.shape[1] // LANE):
        acc = acc + x[:, j * LANE:(j + 1) * LANE]
    return acc


def _row_mean(x):
    return jnp.sum(_lane_tiles_sum(x), axis=-1, keepdims=True) * (1.0 / D)


def _kernel(x_hbm, wqkv_hbm, wo_hbm, w1_hbm, w2_hbm, w3_hbm, w4_hbm, gw_hbm,
            out_hbm,
            x_v, wq_v, wk_v, wv_v, wo_v, w1_v, w2_v, w3_v, w4_v, gw_v,
            ln0_v, w2rs_v, h_v, g_v, mx_v, wqt_v, g_acc, z_acc, m_v, zb_v, obuf,
            isem, osem):
    def x_cp(t):
        if isinstance(t, int) and t < 0:
            return pltpu.make_async_copy(x_hbm.at[pl.ds(0, T0)], x_v.at[pl.ds(0, T0)], isem.at[NW])
        return pltpu.make_async_copy(x_hbm.at[pl.ds(T0 + t * T1, T1)], x_v.at[pl.ds(T0 + t * T1, T1)],
                                     isem.at[NW + 1 + t])

    srcs = [
        ("gw", gw_hbm, gw_v),
        ("wka", wqkv_hbm.at[pl.ds(0, KS), pl.ds(D, D)], wk_v.at[pl.ds(0, KS)]),
        ("wkb", wqkv_hbm.at[pl.ds(KS, D - KS), pl.ds(D, D)], wk_v.at[pl.ds(KS, D - KS)]),
        ("w1", w1_hbm, w1_v), ("w2", w2_hbm, w2_v),
        ("wv", wqkv_hbm.at[:, pl.ds(2 * D, D)], wv_v), ("wo", wo_hbm, wo_v),
        ("wq", wqkv_hbm.at[:, pl.ds(0, D)], wq_v), ("w3", w3_hbm, w3_v), ("w4", w4_hbm, w4_v),
    ]
    wcp = {nm: pltpu.make_async_copy(src, dst, isem.at[i]) for i, (nm, src, dst) in enumerate(srcs)}
    wcp["gw"].start()
    x_cp(-1).start()
    for nm in ("wka", "wkb", "w1"):
        wcp[nm].start()
    for t in range(N1):
        x_cp(t).start()
    for nm in ("wv", "wo", "wq", "w2", "w3", "w4"):
        wcp[nm].start()

    h_v[pl.ds(0, HP * NJ), :] = jnp.zeros((HP * NJ, LANE), F32)
    h_v[pl.ds((HP + S) * NJ, HP * NJ), :] = jnp.zeros((HP * NJ, LANE), F32)

    def store_h(r, n, h):
        for j in range(NJ):
            h_v[pl.ds((HP + r) * NJ + j, n, stride=NJ), :] = h[:, j * LANE:(j + 1) * LANE]

    def shifted_h(r, n):
        lane = jax.lax.broadcasted_iota(jnp.int32, (n, LANE), 1)

        def sh(k, j):
            return h_v[pl.ds((HP + r + k) * NJ + j, n, stride=NJ), :]

        return jnp.concatenate([
            sh(-1, 0),
            jnp.where(lane < 32, sh(-1, 1), sh(1, 1)),
            jnp.where(lane < 64, sh(1, 2), sh(-2, 2)),
            jnp.where(lane < 96, sh(-2, 3), sh(2, 3)),
            sh(2, 4)], axis=1)

    def row_stats(r0, n, xb):
        xf = xb.astype(F32)
        m = _row_mean(xf)
        xc = xf - m
        rs = jax.lax.rsqrt(_row_mean(xc * xc) + 1e-5)
        gw = gw_v[...].astype(F32)
        acc = xf[:, 0:LANE] * gw[0:1, :]
        for j in range(1, NJ):
            acc = acc + xf[:, j * LANE:(j + 1) * LANE] * gw[j:j + 1, :]
        gate = _sigmoid(jnp.sum(acc, axis=-1, keepdims=True))
        g_v[pl.ds(r0, n), :] = jnp.broadcast_to(gate, (n, LANE))
        mx_v[pl.ds(r0, n), :] = jnp.broadcast_to(m, (n, LANE))
        return (xf * rs - m * rs).astype(BF)

    def col_sums8(pk):
        return jnp.sum(pk.reshape(pk.shape[0] // 8, 8, D), axis=0)

    x_cp(-1).wait()
    wcp["gw"].wait()
    x0 = x_v[pl.ds(0, T0), :]
    ln0_v[...] = row_stats(0, T0, x0)
    wcp["wka"].wait()
    k0 = _dot_rows(x0[:, :KS], wk_v[0:KS, :], 4)
    wcp["wkb"].wait()
    pk0 = _phi(k0 + _dot_rows(x0[:, KS:], wk_v[KS:D, :], 4))
    z_acc[...] = col_sums8(pk0)
    g_acc[...] = _dot_rows(pk0.astype(BF).T, x0, 2)
    wcp["w1"].wait()

    def phase1(t, carry):
        r0 = pl.multiple_of(T0 + t * T1, LANE)
        x_cp(t).wait()
        xb = x_v[pl.ds(r0, T1), :]
        pk = _phi(_dot(xb, wk_v[...]))
        z_acc[...] += col_sums8(pk)
        pkt = pk.astype(BF).T
        ln = row_stats(r0, T1, xb)
        store_h(r0, T1, _gelu(_dot(ln, w1_v[...])))
        g_acc[...] += _dot(pkt, xb)
        return carry

    jax.lax.fori_loop(0, N1, phase1, 0)

    for nm in ("wv", "wo", "wq", "w2", "w3", "w4"):
        wcp[nm].wait()
    z = jnp.sum(z_acc[...], axis=0, keepdims=True)
    zb_v[...] = jnp.broadcast_to(z, (LANE, D)).T
    wqt_v[...] = wq_v[...].T
    for c in range(NJ):
        blk = _lane_tiles_sum(w2_v[pl.ds(c * LANE, LANE), :].astype(F32))
        w2rs_v[:, pl.ds(c * LANE, LANE)] = jnp.sum(blk.T.reshape(LANE // 8, 8, LANE), axis=0)
    kvm = []
    for j, (lo, hi) in enumerate(BANDS):
        n = hi - lo
        rr = jax.lax.broadcasted_iota(jnp.int32, (n, LANE), 0) + lo
        cc = jax.lax.broadcasted_iota(jnp.int32, (n, LANE), 1) + j * LANE
        kv = _dot(g_acc[pl.ds(lo, n), :].astype(BF), wv_v[:, pl.ds(j * LANE, LANE)])
        kvm.append(jnp.where(_head_of(rr) == _head_of(cc), kv, 0.0).astype(BF))
    store_h(0, T0, _gelu(_dot(ln0_v[...], w1_v[...])))
    parts = [_dot(kvm[j], wo_v[pl.ds(j * LANE, LANE), :]) for j in range(NJ)]
    edges = sorted(set([lo for lo, _ in BANDS] + [hi for _, hi in BANDS]))
    for a, b in zip(edges[:-1], edges[1:]):
        acc = None
        for j, (lo, hi) in enumerate(BANDS):
            if lo <= a and b <= hi:
                p = parts[j][a - lo:b - lo]
                acc = p if acc is None else acc + p
        m_v[pl.ds(a, b - a), :] = acc.astype(BF)

    pieces = [(c * LANE, 0, T2) for c in range(NJ - 1)] + [((NJ - 1) * LANE, r, OR) for r in range(0, T2, OR)]
    NP = H // 2
    lo4 = jax.lax.broadcasted_iota(jnp.int32, (NP, 8, T2), 1) < 4

    def all_sublanes_sum(a):
        a = a + pltpu.roll(a, 4, 1)
        a = a + pltpu.roll(a, 2, 1)
        return a + pltpu.roll(a, 1, 1)

    def recip(d):
        r = pl.reciprocal(d, approx=True)
        return r * (2.0 - d * r)

    def phase2(t, carry):
        r0 = pl.multiple_of(t * T2, T2)
        xb = x_v[pl.ds(r0, T2), :]
        pq = _phi(_dot_nt(wqt_v[...], xb))
        tz = (pq * jnp.concatenate([zb_v[...]] * (T2 // LANE), axis=1)).reshape(NP, 5, 8, T2)
        p4 = pq.reshape(NP, 5, 8, T2)
        ra = recip(all_sublanes_sum(tz[:, 0] + tz[:, 1] + jnp.where(lo4, tz[:, 2], 0.0)) + 1e-6)
        rb = recip(all_sublanes_sum(tz[:, 3] + tz[:, 4] + jnp.where(lo4, 0.0, tz[:, 2])) + 1e-6)
        pqn = jnp.stack([p4[:, 0] * ra, p4[:, 1] * ra, p4[:, 2] * jnp.where(lo4, ra, rb),
                         p4[:, 3] * rb, p4[:, 4] * rb], axis=1).reshape(D, T2).astype(BF)
        hs = shifted_h(r0, T2).astype(BF)
        w2rs = jnp.sum(w2rs_v[...], axis=0, keepdims=True)
        m = mx_v[pl.ds(r0, T2), :] + _row_mean(hs.astype(F32) * w2rs)
        xc = (xb.astype(F32) - jnp.concatenate([m] * NJ, axis=1)) + _dot(hs, w2_v[...])
        ln = xc.astype(BF)
        rs = jax.lax.rsqrt(_row_mean(xc * xc) + 1e-5)
        a = _dot_tn(pqn, m_v[...])
        h3l = _gelu(_dot_nt(w3_v[FM:F, :], ln).T * rs).astype(BF)
        h3m = _gelu(_dot_nt(ln, w3_v[0:FM, :]) * rs).astype(BF)
        bm = xc + _dot(jnp.concatenate([h3m, h3l], axis=1), w4_v[...])
        g = g_v[pl.ds(r0, T2), :]
        for c0, rr, nr in pieces:
            b = bm[rr:rr + nr, c0:c0 + LANE] + m[rr:rr + nr]
            obuf[pl.ds(r0 + rr, nr), pl.ds(c0, LANE)] = (
                b + g[rr:rr + nr] * (a[rr:rr + nr, c0:c0 + LANE] - b)).astype(BF)
            pltpu.make_async_copy(obuf.at[pl.ds(r0 + rr, nr), pl.ds(c0, LANE)],
                                  out_hbm.at[pl.ds(r0 + rr, nr), pl.ds(c0, LANE)], osem.at[0]).start()
        return carry

    jax.lax.fori_loop(0, N2, phase2, 0)
    pltpu.make_async_copy(obuf, out_hbm, osem.at[0]).wait()


@jax.jit
def pallas_gated_mix__linear_attn_block__mixer_s_mlp__prompt_kernel(
        A_x, A_wqkv, A_wo, B_x, B_w1, B_w2, B_w3, B_w4, gate_w):
    del B_x
    hbm = pl.BlockSpec(memory_space=pltpu.HBM)
    out = pl.pallas_call(
        _kernel,
        out_shape=jax.ShapeDtypeStruct((S, D), BF),
        in_specs=[hbm] * 8,
        out_specs=hbm,
        scratch_shapes=[
            pltpu.VMEM((S, D), BF),
            pltpu.VMEM((D, D), BF), pltpu.VMEM((D, D), BF), pltpu.VMEM((D, D), BF),
            pltpu.VMEM((D, D), BF), pltpu.VMEM((D, D), BF), pltpu.VMEM((D, D), BF),
            pltpu.VMEM((F, D), BF), pltpu.VMEM((F, D), BF),
            pltpu.VMEM((NJ, LANE), BF),
            pltpu.VMEM((T0, D), BF),
            pltpu.VMEM((8, D), F32),
            pltpu.VMEM(((HP + S + HP) * NJ, LANE), F32),
            pltpu.VMEM((S, LANE), F32), pltpu.VMEM((S, LANE), F32),
            pltpu.VMEM((D, D), BF),
            pltpu.VMEM((D, D), F32), pltpu.VMEM((8, D), F32),
            pltpu.VMEM((D, D), BF), pltpu.VMEM((D, LANE), F32),
            pltpu.VMEM((S, D), BF),
            pltpu.SemaphoreType.DMA((NW + 1 + N1,)),
            pltpu.SemaphoreType.DMA((1,)),
        ],
        compiler_params=pltpu.CompilerParams(
            vmem_limit_bytes=100 * 1024 * 1024,
            disable_bounds_checks=True,
            disable_semaphore_checks=True,
        ),
        name="gmix",
    )(A_x.reshape(S, D), A_wqkv, A_wo, B_w1, B_w2, B_w3.T, B_w4, gate_w.reshape(NJ, LANE))
    return out.reshape(1, S, D)
```
